```python
import jax
import jax.numpy as jnp

def _softmax(x, axis=-1):
    return jax.nn.softmax(x, axis=axis)

def _gelu(x):
    return jax.nn.gelu(x, approximate=True)

def _silu(x):
    return jax.nn.silu(x)

def _sigmoid(x):
    return jax.nn.sigmoid(x)

def _layernorm(x, axis=-1, eps=1e-05):
    m = jnp.mean(x, axis=axis, keepdims=True)
    v = jnp.var(x, axis=axis, keepdims=True)
    return (x - m) / jnp.sqrt(v + eps)

def _scatter_add(tgt, idx, src, axis=0):
    return tgt.at[idx].add(src)

def _segment_sum(src, seg, n):
    return jax.ops.segment_sum(src, seg, n)

class _Rng:

    def __init__(self, key):
        self._k = key

    def _next(self):
        self._k, sub = jax.random.split(self._k)
        return sub

    def normal(self, shape):
        return jax.random.normal(self._next(), shape, dtype=jnp.bfloat16)

    def randint(self, lo, hi, shape):
        return jax.random.randint(self._next(), shape, lo, hi, dtype=jnp.int32)

    def uniform(self, shape, lo=0.0, hi=1.0):
        return jax.random.uniform(self._next(), shape, jnp.bfloat16, lo, hi)

    def permutation(self, n):
        return jax.random.permutation(self._next(), n)
kernel_name = 'adaLN_cond__linear_kernel_hedgehog__moe_arch_mod__prompt'

def setup_inputs():
    _rng = _Rng(jax.random.key(int.from_bytes(__import__("os").urandom(4), "little")))
    _w = lambda a: (lambda t: t.astype(jnp.bfloat16) if jnp.issubdtype(t.dtype, jnp.floating) else t)(jnp.asarray(a))

    def _A_setup():
        B, S, D, H = (1, 2048, 1024, 32)
        Dh = D // H
        return {'x': _w((lambda *s: _rng.normal(s) * 0.05)(B, S, D)), 'wqkv': _w((lambda *s: _rng.normal(s) * 0.05)(D, 3 * D)), 'w_phi': _w((lambda *s: _rng.normal(s) * 0.05)(H, Dh, Dh) * Dh ** (-0.5)), 'wo': _w((lambda *s: _rng.normal(s) * 0.05)(D, D))}
    _A_in = _A_setup()

    def _B_setup():
        B, S, D, F, C = (1, 2048, 1024, 3584, 2)
        return {'x': _w((lambda *s: _rng.normal(s) * 0.05)(B, S, D)), 'w_r': _w((lambda *s: _rng.normal(s) * 0.05)(D)), 'w_gate': _w((lambda *s: _rng.normal(s) * 0.05)(D, F)), 'w_up': _w((lambda *s: _rng.normal(s) * 0.05)(D, F)), 'w_down': _w((lambda *s: _rng.normal(s) * 0.05)(F, D))}
    _B_in = _B_setup()
    return {'A_x': _A_in['x'], 'A_wqkv': _A_in['wqkv'], 'A_w_phi': _A_in['w_phi'], 'A_wo': _A_in['wo'], 'B_x': _B_in['x'], 'B_w_r': _B_in['w_r'], 'B_w_gate': _B_in['w_gate'], 'B_w_up': _B_in['w_up'], 'B_w_down': _B_in['w_down'], 'c': _w((lambda *s: _rng.normal(s) * 0.05)(1, 1024)), 'w_mod': _w((lambda *s: _rng.normal(s) * 0.05)(1024, 6 * 1024) * 1024 ** (-0.5))}

def reference(A_x, A_wqkv, A_w_phi, A_wo, B_x, B_w_r, B_w_gate, B_w_up, B_w_down, c, w_mod):

    def _A_ref(x, wqkv, w_phi, wo):
        B, S, D = x.shape
        H = 32
        Dh = D // H
        qkv = (lambda x, *d: x.transpose(*d))((x @ wqkv).reshape(B, S, 3, H, Dh), 2, 0, 3, 1, 4)
        q, k, v = (qkv[0], qkv[1], qkv[2])
        pq = jnp.einsum('bhsd,hdf->bhsf', q, w_phi)
        pk = jnp.einsum('bhsd,hdf->bhsf', k, w_phi)
        phi_q = jnp.concatenate([_softmax(pq, axis=-1), _softmax(-pq, axis=-1)], axis=-1)
        phi_k = jnp.concatenate([_softmax(pk, axis=-1), _softmax(-pk, axis=-1)], axis=-1)
        kv = jnp.einsum('bhsf,bhsd->bhfd', phi_k, v)
        z = jnp.einsum('bhsf->bhf', phi_k)
        num = jnp.einsum('bhqf,bhfd->bhqd', phi_q, kv)
        den = jnp.einsum('bhqf,bhf->bhq', phi_q, z)[..., None] + 1e-06
        o = num / den
        return (lambda x, *d: x.transpose(*d))(o, 0, 2, 1, 3).reshape(B, S, D) @ wo

    def _B_ref(x, w_r, w_gate, w_up, w_down):
        B, S, D = x.shape
        C = 2
        r = x @ w_r
        idx = jnp.argsort(-r, axis=-1)[:, :C]
        idx_e = jnp.repeat(idx.reshape(B, C, 1), D, axis=2)
        x_sel = jnp.take_along_axis(x, idx_e, axis=1)
        g = _silu(x_sel @ w_gate)
        u = x_sel @ w_up
        y = g * u @ w_down
        r_sel = _sigmoid(jnp.take_along_axis(r, idx, axis=1))
        y = y * r_sel.reshape(B, C, 1)
        b_off = (jnp.arange(B) * S).reshape(B, 1)
        flat_idx = (idx + b_off).reshape(B * C)
        zero = (x * 0.0).reshape(B * S, D)
        upd = _scatter_add(zero, flat_idx, y.reshape(B * C, D), axis=0)
        return x + upd.reshape(B, S, D)
    x = A_x
    mod = (_silu(c) @ w_mod).reshape(c.shape[0], 6, 1, -1)
    sa, ca, ga, sb, cb, gb = (mod[:, 0].copy(), mod[:, 1].copy(), mod[:, 2].copy(), mod[:, 3].copy(), mod[:, 4].copy(), mod[:, 5].copy())
    h = _layernorm(x, axis=-1) * (1 + ca) + sa
    x = x + ga * _A_ref(h, A_wqkv, A_w_phi, A_wo)
    h = _layernorm(x, axis=-1) * (1 + cb) + sb
    x = x + gb * _B_ref(h, B_w_r, B_w_gate, B_w_up, B_w_down)
    return x
```

```python
import jax
import jax.numpy as jnp
import numpy as np
from jax import lax
from jax.experimental import pallas as pl
from jax.experimental.pallas import tpu as pltpu

S = 2048
D = 1024
H = 32
DH = D // H
F = 3584
LANES = 128
HALF = D // 2
NJ = D // LANES
NF = F // LANES
NP = H // 2
TM = 512
TH = TM // 2
NT = S // TM
LOG2E = float(np.log2(np.e))
LN_EPS = 1e-5
DEN_EPS = 1e-6

BF16 = jnp.bfloat16
F32 = jnp.float32
U32 = jnp.uint32
NN = (((1,), (0,)), ((), ()))
TB = (((1,), (1,)), ((), ()))


def _dot(a, b, dims=NN):
  return lax.dot_general(a, b, dims, preferred_element_type=F32)


def _left_operands(a11, a12, a21, a22):
  return [a11 + a22, a21 + a22, a11, a22, a11 + a12, a21 - a11, a12 - a22]


def _right_operands(b11, b12, b21, b22):
  return [b11 + b22, b11, b12 - b22, b21 - b11, b22, b11 + b12, b21 + b22]


def _tree(op, xs):
  while len(xs) > 1:
    xs = [op(xs[i], xs[i + 1]) if i + 1 < len(xs) else xs[i]
          for i in range(0, len(xs), 2)]
  return xs[0]


def _lane_tiles(x):
  return [x[:, t * LANES:(t + 1) * LANES] for t in range(x.shape[1] // LANES)]


def _assemble(blocks):
  return jnp.concatenate([jnp.concatenate(r, axis=1) for r in blocks], axis=0).astype(BF16)


def _after(x, token):
  if token is None:
    return x
  head = pltpu.bitcast(x[0:8, 0:LANES], U32)
  head = pltpu.bitcast(head | (head & pltpu.bitcast(token, U32)), F32)
  if x.shape[1] > LANES:
    head = jnp.concatenate([head, x[0:8, LANES:]], axis=1)
  return jnp.concatenate([head, x[8:]], axis=0) if x.shape[0] > 8 else head


def _token(*vals):
  tiles = [pltpu.bitcast(v[r:r + 8, l:l + LANES], U32) for v in vals
           for r in range(0, v.shape[0], 8) for l in range(0, v.shape[1], LANES)]
  return _tree(jnp.bitwise_or, tiles)


class _Stream:
  def __init__(self):
    self.budget = 800
    self.urgent = []
    self.relaxed = []
    self.deferred = []
    self.tokens = []

  def later(self, products, fn):
    self.deferred.append([products, fn])

  def product(self, a, b, dims, quiet=False):
    m = _dot(a, b, dims)
    groups = m.shape[0] // 8
    spot = lambda j, n: divmod(j * groups * (m.shape[1] // LANES) // n, groups)
    due = [t for wait, t in self.tokens if wait <= 1]
    self.tokens = [(wait - 1, t) for wait, t in self.tokens if wait > 1]
    if due:
      tiles = [[t[r:r + 8] for r in range(0, m.shape[0], 8)] for t in _lane_tiles(m)]
      for j, token in enumerate(due):
        t, g = spot(j, len(due))
        tiles[t][g] = _after(tiles[t][g], token)
      m = jnp.concatenate([jnp.concatenate(t, axis=0) for t in tiles], axis=1)
    due = [fn for wait, fn in self.deferred if wait <= 1]
    self.deferred = [[wait - 1, fn] for wait, fn in self.deferred if wait > 1]
    for fn in due:
      fn()
    budget = self.budget * m.shape[0] * m.shape[1] * a.shape[1] // (TH * TH * HALF)
    chosen = []
    for queue in () if quiet else (self.urgent, self.relaxed):
      if queue is self.relaxed:
        budget = max(budget, 60)
      while queue and budget >= queue[0][0] // 2:
        budget -= queue[0][0]
        chosen.append(queue.pop(0)[1])
    for j, fn in enumerate(chosen):
      t, g = spot(j, len(chosen))
      token = fn(m[8 * g:8 * g + 8, t * LANES:(t + 1) * LANES])
      if token is not None:
        self.tokens.append((1, token))
    return m

  def flush(self, queue):
    while queue:
      queue.pop(0)[1](None)

  def drain(self):
    while self.urgent or self.deferred:
      self.flush(self.urgent)
      self.flush_deferred()

  def flush_deferred(self):
    while self.deferred:
      self.deferred.pop(0)[1]()

  def block_product(self, left, right, dims, done, rows_first=False, quiet_end=False):
    mul = lambda i: self.product(left[i], right[i], dims)
    m5 = mul(4)
    m3 = mul(2)
    done(0, 1, m3 + m5)
    m4 = mul(3)
    c11 = m4 - m5
    if rows_first:
      m1 = mul(0)
      c11 = c11 + m1
      c22 = m3 + m1
      done(0, 0, c11 + mul(6))
      m2 = mul(1)
      done(1, 0, m2 + m4)
      c22 = c22 - m2
      done(1, 1, c22 + mul(5))
      return
    m2 = mul(1)
    done(1, 0, m2 + m4)
    c22 = m3 - m2
    m1 = mul(0)
    c11 = c11 + m1
    c22 = c22 + m1
    done(0, 0, c11 + mul(6))
    done(1, 1, c22 + self.product(left[5], right[5], dims, quiet_end))


def _normalize(x):
  xc = x - jnp.mean(x, axis=-1, keepdims=True)
  var = jnp.mean(xc * xc, axis=-1, keepdims=True)
  return xc * lax.rsqrt(var + LN_EPS)


def _per_head(op, xs):
  r = _tree(op, xs)
  r = op(r, pltpu.roll(r, 4, 0))
  return op(r, pltpu.roll(r, 2, 0))


def _hedgehog(p):
  xs = [p[8 * i:8 * i + 8] for i in range(p.shape[0] // 8)]
  hi = _per_head(jnp.maximum, xs)
  lo = _per_head(jnp.minimum, xs)
  pos = [jnp.exp2(x - hi) for x in xs]
  neg = [jnp.exp2(lo - x) for x in xs]
  if 1:
    hi = hi + jnp.log2(_per_head(jnp.add, pos))
    lo = lo - jnp.log2(_per_head(jnp.add, neg))
    return [jnp.exp2(x - hi) for x in xs] + [jnp.exp2(lo - x) for x in xs]
  inv_pos = 1.0 / _per_head(jnp.add, pos)
  inv_neg = 1.0 / _per_head(jnp.add, neg)
  return [e * inv_pos for e in pos] + [e * inv_neg for e in neg]


def _kernel(x_hbm, wqkv_hbm, wphi_hbm, wo_hbm, wr_hbm, wg_hbm, wu_hbm, wd_hbm,
            c_hbm, wmod_hbm, out_hbm,
            x_v, wqkv_v, wphi_v, wo_v, wr_v, wg_v, wu_v, wd_v, c_v, wmod_v,
            wshift_v, wscale_v, norm_v, first_v, h2_v, out_v, patch_v, sem):
  sems = iter(range(sem.shape[0]))

  def copy(src, dst):
    return pltpu.make_async_copy(src, dst, sem.at[next(sems)])

  def slab_copies(src, dst, first=0, which=None):
    k = next(sems)
    return [pltpu.make_async_copy(src.at[:, pl.ds((first + j) * LANES, LANES)], dst.at[j],
                                  sem.at[k]) for j in which or range(dst.shape[0])]

  def slabs(ref, which=None):
    return jnp.concatenate([ref[j] for j in which or range(ref.shape[0])], axis=1)

  cp_c = copy(c_hbm, c_v)
  cp_phi = copy(wphi_hbm, wphi_v)
  cp_wr = copy(wr_hbm, wr_v)
  cp_wq, cp_wk = [
      [slab_copies(wqkv_hbm, wqkv_v.at[i], i * NJ, (2 * u, 2 * u + 1, 2 * u + 4, 2 * u + 5))
       for u in range(2)] for i in range(2)]
  cp_wv = [slab_copies(wqkv_hbm, wqkv_v.at[2], 2 * NJ, which)
           for which in ((0, 1, 4, 5), (2, 6), (3, 7))]
  cp_shift = slab_copies(wmod_hbm, wshift_v)
  cp_scale = [slab_copies(wmod_hbm, wscale_v, NJ, (j, j + 4)) for j in range(4)]
  cp_mod = [copy(wmod_hbm.at[:, pl.ds(i * D, D)], wmod_v.at[i - 2]) for i in range(2, 6)]
  cp_x = [copy(x_hbm.at[pl.ds(i * TM, TM)], x_v.at[pl.ds(i * TM, TM)]) for i in range(NT)]
  cp_wo = copy(wo_hbm, wo_v)
  cp_wg = slab_copies(wg_hbm, wg_v)
  cp_wu = slab_copies(wu_hbm, wu_v)
  cp_wd = slab_copies(wd_hbm, wd_v)
  cp_out = [copy(out_v.at[pl.ds(i * TH, TH)], out_hbm.at[pl.ds(i * TH, TH)])
            for i in range(S // TH)]
  patch_sems = [next(sems), next(sems)]
  cp_late = cp_wq[0] + cp_wq[1] + [cp_wr] + cp_mod + [cp_wo]

  cp_scale[3] = cp_wv[1] + cp_scale[3]
  for cp in ([cp_c] + cp_wv[0] + [cp_x[0]] + sum(cp_scale, []) + cp_wv[2]
             + [cp_phi] + cp_wk[0] + cp_shift + [cp_x[1]] + cp_wk[1] + cp_x[2:] + cp_late):
    cp.start()

  stream = _Stream()
  mod = {}

  def block_diagonals():
    row = lax.broadcasted_iota(jnp.int32, (LANES, DH), 0)
    col = lax.broadcasted_iota(jnp.int32, (LANES, DH), 1)
    pick = jnp.where((row % 64) // 2 == col, 1.0, 0.0).astype(BF16)
    row = lax.broadcasted_iota(jnp.int32, (LANES, LANES), 0)
    col = lax.broadcasted_iota(jnp.int32, (LANES, LANES), 1)
    own_head = (row // 64) * 2 + row % 2 == col // DH
    return [jnp.where(own_head, _dot(pick, wphi_v[g * LANES:(g + 1) * LANES, :], TB),
                      0.0).astype(BF16) for g in range(NJ)]

  def weight_operands(parts):
    return [_assemble([[p[i] for p in row] for row in parts]) for i in range(7)]

  def value_weight(g, j):
    return wqkv_v[2, g, j * LANES:(j + 1) * LANES, :].astype(F32).T

  def value_weight_parts(g, j):
    return _left_operands(value_weight(g, j), value_weight(g, j + 4),
                          value_weight(g + 4, j), value_weight(g + 4, j + 4))

  def fold_phi(which, u):
    parts = []
    for g in (2 * u, 2 * u + 1):
      top, bot = [_lane_tiles(LOG2E * stream.product(
          bd[k], wqkv_v[which, k], TB)) for k in (g, g + 4)]
      parts.append([_left_operands(top[j], top[j + 4], bot[j], bot[j + 4]) for j in range(4)])
    return weight_operands(parts)

  def load_f32(ref, start):
    return ref[pl.ds(start, 16), :].astype(F32)

  wo_parts = []

  def out_weight_piece(r, token):
    top = _after(load_f32(wo_v, r), token)
    bot = load_f32(wo_v, HALF + r)
    ops = _right_operands(top[:, :HALF], top[:, HALF:], bot[:, :HALF], bot[:, HALF:])
    wo_parts.append(ops)
    return _token(ops[0], ops[2], ops[5])

  def modulation_pieces(i):
    acc = []
    def piece(k, token):
      w = load_f32(wmod_v.at[i - 2], k)
      p = w * jnp.tile(_after(silu_col[k:k + 16], token), (1, NJ))
      p = p[0:8] + p[8:16]
      acc[:] = [acc[0] + p] if acc else [p]
      if k + 16 == D:
        mod[i] = jnp.sum(acc[0], axis=0, keepdims=True)
      return _token(acc[0]) if k % 64 == 48 else None
    return [(60, lambda t, k=k: piece(k, t)) for k in range(0, D, 16)]

  h_parts = [[] for _ in range(NT)]

  def modulate(i, top, bot):
    scale = 1.0 + mod[1]
    top = top * scale + mod[0]
    bot = bot * scale + mod[0]
    ops = _right_operands(top[:, :HALF], bot[:, :HALF], top[:, HALF:], bot[:, HALF:])
    h_parts[i].append(ops)
    return _token(ops[5], ops[6])

  def normalized_rows(start, token=None):
    return _normalize(_after(load_f32(x_v, start), token))

  def prenorm_pieces(i):
    top = []
    def first(r, token):
      top.append(normalized_rows(i * TM + r, token))
    def second(r, token):
      return modulate(i, top.pop(), normalized_rows(i * TM + TH + r, token))
    return [(cost, lambda t, r=r, f=f: f(r, t))
            for r in range(0, TH, 16) for cost, f in ((120, first), (270, second))]

  def h_operands(i):
    return [_assemble([[part[k]] for part in h_parts[i]]) for k in range(7)]

  def columns(row):
    return jnp.concatenate(
        [jnp.broadcast_to(t[0:1], (LANES, LANES)).T for t in _lane_tiles(row)], axis=0)

  cp_c.wait()
  c = jnp.broadcast_to(c_v[...].astype(F32), (16, D))
  silu_c = (c * jax.nn.sigmoid(c)).astype(BF16)
  silu_col = columns(silu_c.astype(F32))

  first_groups = (0, 1, 4, 5)
  for cp in cp_wv[0]:
    cp.wait()
  first_wv = {(g, j): value_weight(g, j) for g in first_groups for j in range(NJ)}

  cp_x[0].wait()
  for r in range(0, TM, 16):
    norm_v[pl.ds(r, 16), :] = normalized_rows(r)

  scales = [None] * NJ
  first_values = None
  for j in range(4):
    for cp in cp_scale[j]:
      cp.wait()
    both = _dot(silu_c, slabs(wscale_v, (j, j + 4)))
    scales[j], scales[j + 4] = _lane_tiles(both[0:1])
    lo, hi = [norm_v[0:TM, t * LANES:(t + 1) * LANES] * (1.0 + scales[t]) for t in (j, j + 4)]
    for k, op in enumerate(_right_operands(lo[:TH], lo[TH:], hi[:TH], hi[TH:])):
      first_v[1, k, :, pl.ds(j * LANES, LANES)] = op.astype(BF16)
    term = _dot(_assemble([[first_wv[g, j], first_wv[g, j + 4]] for g in first_groups]),
                _assemble([[lo, hi]]), TB)
    first_values = term if j == 0 else _after(first_values, both[0:8, 0:LANES]) + term
  mod[1] = jnp.concatenate(scales, axis=1)

  kv = [None] * NP
  z = [None] * NP
  h = []
  keys, values = {}, {}
  width = TH if 0 else LANES

  def pairs_of(u, row):
    return [(8 * row + 4 * u + k, 64 * k) for k in range(4)]

  def accumulate(acc, i, val):
    acc[i] = val if acc[i] is None else acc[i] + val

  def feature_pieces(u, row, block, cost, use):
    for pair, r in pairs_of(u, row):
      parts = []
      def piece(token, pair=pair, r=r, parts=parts):
        lo = len(parts) * width
        parts.append(_hedgehog(_after(block[r:r + 64, lo:lo + width], token)))
        use(pair, parts)
        return _token(parts[-1][7], parts[-1][15]) if 1 else None
      stream.urgent += [(cost * width // LANES, piece)] * (TH // width)

  def combine(n, pair):
    if (n, pair) in keys and (n, pair) in values:
      def run():
        v = values[n, pair]
        if n < 2:
          v = v + jnp.tile(value_shift[64 * pair:64 * pair + 64], (1, TH // LANES))
        accumulate(kv, pair, _dot(v.astype(BF16), keys[n, pair], TB))
      stream.later(1, run)

  def keys_done(i, u, row, col, block):
    def use(pair, parts):
      if len(parts) == TH // width:
        phi = jnp.concatenate([jnp.concatenate(p, axis=0) for p in parts], axis=1)
        accumulate(z, pair, _tree(jnp.add, _lane_tiles(phi)))
        keys[2 * i + col, pair] = phi.astype(BF16)
        combine(2 * i + col, pair)
    feature_pieces(u, row, block, 125, use)

  def values_done(i, u, row, col, block):
    for pair, r in pairs_of(u, row):
      values[2 * i + col, pair] = block[r:r + 64]
      combine(2 * i + col, pair)

  def project(w, u, right, done, i, quiet_end=False):
    stream.block_product(w[u], right, TB, lambda *a: done(i, u, *a),
                         quiet_end=quiet_end and 0)

  for row in range(2):
    for col in range(2):
      values_done(0, 0, row, col, first_values[row * TH:(row + 1) * TH, col * TH:(col + 1) * TH])
  def store_value_weights(c):
    for j in range(4):
      for k, op in enumerate(value_weight_parts(2 + c, j)):
        first_v[0, k, pl.ds(c * LANES, LANES), pl.ds(j * LANES, LANES)] = op.astype(BF16)

  store_value_weights(0)
  for cp in cp_wv[2] + [cp_phi]:
    cp.wait()
  store_value_weights(1)
  bd = block_diagonals()
  wv = [None, [first_v[0, k] for k in range(7)]]
  wv_parts = [[[], []]]

  def first_wv_piece(g, j, token):
    wv_parts[0][g].append(_left_operands(
        _after(first_wv[g, j], token), first_wv[g, j + 4],
        first_wv[g + 4, j], first_wv[g + 4, j + 4]))

  stream.relaxed += [(100, lambda t, g=g, j=j: first_wv_piece(g, j, t))
                     for g in range(2) for j in range(4)]
  project(wv, 1, [first_v[1, k] for k in range(7)], values_done, 0)
  stream.flush(stream.relaxed)

  for cp in cp_wk[0]:
    cp.wait()
  wk = [fold_phi(1, 0)]

  for cp in cp_shift:
    cp.wait()
  shift = _dot(silu_c, slabs(wshift_v))
  mod[0] = shift[0:1]
  value_shift = columns(_dot(shift.astype(BF16), slabs(wqkv_v.at[2])))
  for r in range(0, TH, 16):
    modulate(0, norm_v[pl.ds(r, 16), :], norm_v[pl.ds(TH + r, 16), :])
  h.append(h_operands(0))
  project(wk, 0, h[0], keys_done, 0)

  for cp in [cp_x[1]] + cp_wk[1]:
    cp.wait()
  stream.urgent[:0] = prenorm_pieces(1)
  stream.budget = 800
  wk.append(fold_phi(1, 1))
  project(wk, 1, h[0], keys_done, 0)
  while len(h_parts[1]) < TH // 16:
    stream.urgent.pop(0)[1](None)
  stream.budget = 800

  long_term = [p for k in range(2, 6) for p in modulation_pieces(k)]
  long_term += [(150, lambda t, r=r: out_weight_piece(r, t)) for r in range(0, HALF, 16)]

  def late_weights():
    for cp in cp_late:
      cp.wait()
    for cp in cp_wu + cp_wd:
      cp.start()
    stream.relaxed += long_term

  for i in range(1, NT):
    h.append(h_operands(i))
    if i == 1:
      for cp in cp_x[2:]:
        cp.wait()
      for cp in cp_wg:
        cp.start()
      wv[0] = weight_operands(wv_parts[0])
    if i + 1 < NT:
      stream.relaxed[:0] = prenorm_pieces(i + 1)
    for u in range(2):
      project(wv, u, h[i], values_done, i)
    if i == 2 and 1 == 1:
      late_weights()
    project(wk, 0, h[i], keys_done, i)
    if i == 2 and 1 == 0:
      late_weights()
    project(wk, 1, h[i], keys_done, i)
    while i + 1 < NT and len(h_parts[i + 1]) < TH // 16:
      stream.relaxed.pop(0)[1](None)

  wq = [fold_phi(0, u) for u in range(2)]
  stream.drain()
  wo = []

  row = lax.broadcasted_iota(jnp.int32, (64, LANES), 0)
  col = lax.broadcasted_iota(jnp.int32, (64, LANES), 1)
  own_head = row // DH == col % 2
  kv = [jnp.where(own_head, t, 0.0).astype(BF16) for t in kv]
  z = [jnp.broadcast_to(jnp.sum(t, axis=1, keepdims=True), (LANES, LANES)) for t in z]

  w_r = jnp.concatenate([wr_v[j:j + 1, :].astype(F32) for j in range(NJ)], axis=1)
  o_t = {}
  o_parts = {}
  sublane = lax.broadcasted_iota(jnp.int32, (8, LANES), 0)
  best = [jnp.full((8, LANES), -jnp.inf, F32), jnp.full((8, LANES), S, jnp.int32)] * 2

  def o_piece(n, g, token):
    lo, hi = [_lane_tiles(_after(
        jnp.concatenate(o_t[n, 2 * k] + o_t[n, 2 * k + 1], axis=0), token)) for k in (g, g + 4)]
    o_parts[n, g] = _left_operands(lo[0].T, hi[0].T, lo[1].T, hi[1].T)
    return _token(o_parts[n, g][4][-8:], o_parts[n, g][1][-8:]) if 0 else None

  def queries_done(i, u, row, col, block):
    n = 2 * i + col
    inv = {}
    def use(pair, parts):
      den = _per_head(jnp.add, [p * jnp.tile(z[pair][8 * k:8 * k + 8], (1, width // LANES))
                                for k, p in enumerate(parts[-1])])
      inv.setdefault(pair, []).append(1.0 / (den + DEN_EPS))
      if len(parts) < TH // width:
        return
      phi = _assemble([[jnp.concatenate(p, axis=0) for p in parts]])
      def run():
        num = _dot(kv[pair], phi)
        scale = jnp.concatenate(inv[pair], axis=1)
        o_t[n, pair] = [num[0:DH] * scale[0:1], num[DH:2 * DH] * scale[1:2]]
        g = pair // 2 % 4
        if all((n, 2 * k + j) in o_t for k in (g, g + 4) for j in range(2)):
          stream.urgent.append((150, lambda t: o_piece(n, g, t)))
      stream.later(1, run)
    feature_pieces(u, row, block, 160, use)

  def finish_rows(start, attn, token):
    rows = pl.ds(start, 16)
    x1 = load_f32(x_v, start) + mod[2] * _after(attn, token)
    h2 = _normalize(x1) * (1.0 + mod[4]) + mod[3]
    h2_v[rows, :] = h2.astype(BF16)
    out_v[rows, :] = (x1 + mod[5] * h2).astype(BF16)
    score = jnp.broadcast_to(jnp.sum(h2 * w_r, axis=1, keepdims=True), (16, LANES))
    for k in (0, 8):
      r, idx = score[k:k + 8], sublane + (start + k)
      m1, i1, m2, i2 = best
      over1, over2 = r > m1, r > m2
      best[:] = [jnp.where(over1, r, m1), jnp.where(over1, idx, i1),
                 jnp.where(over1, m1, jnp.where(over2, r, m2)),
                 jnp.where(over1, i1, jnp.where(over2, idx, i2))]
    if (start + 16) % TH == 0:
      cp_out[start // TH].start()
    return best[2] if 1 else None

  def output(n):
    if any((n, g) not in o_parts for g in range(4)):
      stream.drain()
    if not wo:
      stream.flush(stream.relaxed)
      wo.extend(_assemble([[part[k]] for part in wo_parts]) for k in range(7))
    blocks = {}
    def done(row, col, block):
      blocks[row, col] = block
      if (row, 1 - col) in blocks:
        for r in range(0, TH // 2, 16):
          attn = jnp.concatenate([blocks[row, 0][r:r + 16], blocks[row, 1][r:r + 16]], axis=1)
          start = n * TH + row * (TH // 2) + r
          stream.urgent.append((260, lambda t, s=start, a=attn: finish_rows(s, a, t)))
    left = [_assemble([[o_parts[n, g][k] for g in range(4)]]) for k in range(7)]
    if n == 2 * NT - 1:
      stream.budget = 1000
    stream.block_product(left, wo, NN, done, rows_first=n >= 2 * NT - 1)

  for i in range(NT + 1):
    for u in range(2):
      if i < NT:
        project(wq, u, h[i], queries_done, i)
      if i > 0 and 0 == 1:
        output(2 * i - 2 + u)
    if i > 0 and 0 == 0:
      output(2 * i - 2)
      output(2 * i - 1)
  stream.drain()

  score = jnp.concatenate([best[0], best[2]], axis=0)
  idx = jnp.concatenate([best[1], best[3]], axis=0)
  m1 = jnp.max(score, axis=0, keepdims=True)
  i1 = jnp.min(jnp.where(score == m1, idx, S), axis=0, keepdims=True)
  score = jnp.where(idx == i1, -jnp.inf, score)
  m2 = jnp.max(score, axis=0, keepdims=True)
  i2 = jnp.min(jnp.where((score == m2) & (idx != i1), idx, S), axis=0, keepdims=True)
  tok1 = jnp.minimum(i1[0, 0], S - 1)
  tok2 = jnp.minimum(i2[0, 0], S - 1)
  sel = lax.broadcasted_iota(jnp.int32, (16, 1), 0)

  def group_of(tok):
    return pl.multiple_of((tok // 16) * 16, 16)

  def row_of(tok):
    rows = h2_v[pl.ds(group_of(tok), 16), :].astype(F32)
    return jnp.sum(jnp.where(group_of(tok) + sel == tok, rows, 0.0), axis=0, keepdims=True)

  h2_b = jnp.where(sel == 0, row_of(tok1), row_of(tok2)).astype(BF16)
  for cp in cp_wg + cp_wu + cp_wd:
    cp.wait()

  def slabs(ref):
    return jnp.concatenate([ref[j] for j in range(ref.shape[0])], axis=1)

  gate = _dot(h2_b, slabs(wg_v))
  up = _dot(h2_b, slabs(wu_v))
  act = (gate * jax.nn.sigmoid(gate) * up).astype(BF16)
  y = _dot(act, slabs(wd_v))
  y = y * jax.nn.sigmoid(jnp.where(sel == 0, m1[:, 0:1], m2[:, 0:1]))
  update = mod[5] * y

  def patch(slot, tok):
    base = group_of(tok)
    blk = out_v[pl.ds(base, 16), :].astype(F32)
    blk = jnp.where(base + sel == tok1, blk + update[0:1], blk)
    blk = jnp.where(base + sel == tok2, blk + update[1:2], blk)
    patch_v[slot] = blk.astype(BF16)
    return pltpu.make_async_copy(patch_v.at[slot], out_hbm.at[pl.ds(base, 16)],
                                 sem.at[patch_sems[slot]])

  cp1 = patch(0, tok1)
  cp2 = patch(1, tok2)
  for cp in cp_out:
    cp.wait()
  cp1.start()

  @pl.when(tok1 // 16 != tok2 // 16)
  def _():
    cp2.start()
    cp2.wait()

  cp1.wait()


@jax.jit
def pallas_adaLN_cond__linear_kernel_hedgehog__moe_arch_mod__prompt_kernel(
    A_x: jax.Array,
    A_wqkv: jax.Array,
    A_w_phi: jax.Array,
    A_wo: jax.Array,
    B_x: jax.Array,
    B_w_r: jax.Array,
    B_w_gate: jax.Array,
    B_w_up: jax.Array,
    B_w_down: jax.Array,
    c: jax.Array,
    w_mod: jax.Array,
):
  del B_x
  scratch = [
      pltpu.VMEM((S, D), BF16),
      pltpu.VMEM((3, NJ, D, LANES), BF16),
      pltpu.VMEM((D, DH), BF16),
      pltpu.VMEM((D, D), BF16),
      pltpu.VMEM((NJ, LANES), BF16),
      pltpu.VMEM((NF, D, LANES), BF16),
      pltpu.VMEM((NF, D, LANES), BF16),
      pltpu.VMEM((NJ, F, LANES), BF16),
      pltpu.VMEM((1, D), BF16),
      pltpu.VMEM((4, D, D), BF16),
      pltpu.VMEM((NJ, D, LANES), BF16),
      pltpu.VMEM((NJ, D, LANES), BF16),
      pltpu.VMEM((TM, D), F32),
      pltpu.VMEM((2, 7, TH, HALF), BF16),
      pltpu.VMEM((S, D), BF16),
      pltpu.VMEM((S, D), BF16),
      pltpu.VMEM((2, 16, D), BF16),
      pltpu.SemaphoreType.DMA((40,)),
  ]
  flags = {}
  if 0:
    flags["XLA_TPU_EVENLY_DISTRIBUTE_CRITICAL_NODES"] = True
  if 0:
    flags["XLA_TPU_RESCHEDULE_DMA_DONES"] = True
  out = pl.pallas_call(
      _kernel,
      out_shape=jax.ShapeDtypeStruct((S, D), BF16),
      in_specs=[pl.BlockSpec(memory_space=pl.ANY)] * 10,
      out_specs=pl.BlockSpec(memory_space=pl.ANY),
      scratch_shapes=scratch,
      compiler_params=pltpu.CompilerParams(vmem_limit_bytes=120 * 1024 * 1024, flags=flags),
  )(A_x.reshape(S, D), A_wqkv, A_w_phi.reshape(D, DH), A_wo, B_w_r.reshape(NJ, LANES),
    B_w_gate, B_w_up, B_w_down, c, w_mod)
  return out.reshape(1, S, D)
```

```python
import jax
import jax.numpy as jnp
import numpy as np
from jax import lax
from jax.experimental import pallas as pl
from jax.experimental.pallas import tpu as pltpu

S = 2048
D = 1024
H = 32
DH = D // H
F = 3584
LANES = 128
HALF = D // 2
NJ = D // LANES
NF = F // LANES
NP = H // 2
PAIR = 2 * DH
TM = 512
TH = TM // 2
NT = S // TM
VECTOR_SLABS = 10
RATE = 800
LOG2E = float(np.log2(np.e))
LN_EPS = 1e-5
DEN_EPS = 1e-6

BF16 = jnp.bfloat16
F32 = jnp.float32
U32 = jnp.uint32
NN = (((1,), (0,)), ((), ()))
TB = (((1,), (1,)), ((), ()))


def _dot(a, b, dims=NN):
  return lax.dot_general(a, b, dims, preferred_element_type=F32)


def _left_operands(a11, a12, a21, a22):
  return [a11 + a22, a21 + a22, a11, a22, a11 + a12, a21 - a11, a12 - a22]


def _right_operands(b11, b12, b21, b22):
  return [b11 + b22, b11, b12 - b22, b21 - b11, b22, b11 + b12, b21 + b22]


def _tree(op, xs):
  while len(xs) > 1:
    xs = [op(xs[i], xs[i + 1]) if i + 1 < len(xs) else xs[i]
          for i in range(0, len(xs), 2)]
  return xs[0]


def _lane_tiles(x):
  return [x[:, t * LANES:(t + 1) * LANES] for t in range(x.shape[1] // LANES)]


def _assemble(grid):
  return [jnp.concatenate([jnp.concatenate([b[k] for b in row], axis=1) for row in grid],
                          axis=0).astype(BF16) for k in range(7)]


def _columns(row):
  return jnp.concatenate(
      [jnp.broadcast_to(t[0:1], (LANES, LANES)).T for t in _lane_tiles(row)], axis=0)


def _after(x, token):
  if token is None:
    return x
  head = pltpu.bitcast(x[0:8, 0:LANES], U32)
  head = pltpu.bitcast(head | (head & pltpu.bitcast(token, U32)), F32)
  if x.shape[1] > LANES:
    head = jnp.concatenate([head, x[0:8, LANES:]], axis=1)
  return jnp.concatenate([head, x[8:]], axis=0) if x.shape[0] > 8 else head


def _token(*vals):
  tiles = [pltpu.bitcast(v[r:r + 8, l:l + LANES], U32) for v in vals
           for r in range(0, v.shape[0], 8) for l in range(0, v.shape[1], LANES)]
  return _tree(jnp.bitwise_or, tiles)


class _Stream:
  def __init__(self):
    self.rate = RATE
    self.urgent = []
    self.relaxed = []
    self.deferred = []
    self.tokens = []

  def later(self, products, fn):
    self.deferred.append((products, fn))

  def product(self, a, b, dims):
    m = _dot(a, b, dims)
    groups = m.shape[0] // 8
    spot = lambda j, n: divmod(j * groups * (m.shape[1] // LANES) // n, groups)
    if self.tokens:
      tiles = [[t[r:r + 8] for r in range(0, m.shape[0], 8)] for t in _lane_tiles(m)]
      for j, token in enumerate(self.tokens):
        t, g = spot(j, len(self.tokens))
        tiles[t][g] = _after(tiles[t][g], token)
      m = jnp.concatenate([jnp.concatenate(t, axis=0) for t in tiles], axis=1)
      self.tokens = []
    due = [fn for wait, fn in self.deferred if wait <= 1]
    self.deferred = [(wait - 1, fn) for wait, fn in self.deferred if wait > 1]
    for fn in due:
      fn()
    budget = self.rate * max(m.shape[0], 32) * m.shape[1] * a.shape[1] // (TH * TH * HALF)
    chosen = []
    for queue in (self.urgent, self.relaxed):
      if queue is self.relaxed:
        budget = max(budget, 120)
      while queue and budget >= queue[0][0] // 2:
        budget -= queue[0][0]
        chosen.append(queue.pop(0)[1])
    for j, fn in enumerate(chosen):
      t, g = spot(j, len(chosen))
      token = fn(m[8 * g:8 * g + 8, t * LANES:(t + 1) * LANES])
      if token is not None:
        self.tokens.append(token)
    return m

  def flush(self, queue):
    while queue:
      queue.pop(0)[1](None)

  def drain(self):
    while self.urgent or self.deferred:
      self.flush(self.urgent)
      while self.deferred:
        self.deferred.pop(0)[1]()

  def block_product(self, left, right, dims, done, rows_first=False):
    mul = lambda k: self.product(left[k], right[k], dims)
    m5 = mul(4)
    m3 = mul(2)
    done(0, 1, m3 + m5)
    m4 = mul(3)
    c11 = m4 - m5
    if rows_first:
      m1 = mul(0)
      c11 = c11 + m1
      c22 = m3 + m1
      done(0, 0, c11 + mul(6))
      m2 = mul(1)
      done(1, 0, m2 + m4)
      c22 = c22 - m2
    else:
      m2 = mul(1)
      done(1, 0, m2 + m4)
      c22 = m3 - m2
      m1 = mul(0)
      c11 = c11 + m1
      c22 = c22 + m1
      done(0, 0, c11 + mul(6))
    done(1, 1, c22 + mul(5))


def _normalize(x):
  xc = x - jnp.mean(x, axis=-1, keepdims=True)
  var = jnp.mean(xc * xc, axis=-1, keepdims=True)
  return xc * lax.rsqrt(var + LN_EPS)


def _per_head(op, xs):
  r = _tree(op, xs)
  r = op(r, pltpu.roll(r, 4, 0))
  return op(r, pltpu.roll(r, 2, 0))


def _hedgehog(p):
  xs = [p[8 * i:8 * i + 8] for i in range(p.shape[0] // 8)]
  hi = _per_head(jnp.maximum, xs)
  lo = _per_head(jnp.minimum, xs)
  pos = [jnp.exp2(x - hi) for x in xs]
  neg = [jnp.exp2(lo - x) for x in xs]
  hi = hi + jnp.log2(_per_head(jnp.add, pos))
  lo = lo - jnp.log2(_per_head(jnp.add, neg))
  return [jnp.exp2(x - hi) for x in xs] + [jnp.exp2(lo - x) for x in xs]


def _kernel(x_hbm, wqkv_hbm, wphi_hbm, wo_hbm, wr_hbm, wg_hbm, wu_hbm, wd_hbm,
            c_hbm, wmod_hbm, out_hbm,
            x_v, wqkv_v, wphi_v, wo_v, wr_v, wg_v, wu_v, wd_v, c_v, wmod_v, wshift_v,
            wscale_v, norm_v, first_v, h2_v, out_v, hidden_v, patch_v, sem):
  sems = iter(range(sem.shape[0]))

  def copy(src, dst):
    return pltpu.make_async_copy(src, dst, sem.at[next(sems)])

  def slab_copies(src, dst, first=0, which=None):
    k = next(sems)
    return [pltpu.make_async_copy(src.at[:, pl.ds((first + j) * LANES, LANES)], dst.at[j],
                                  sem.at[k]) for j in which or range(dst.shape[0])]

  def slabs(ref, which=None, rows=slice(None)):
    return jnp.concatenate([ref[j, rows, :] for j in which or range(ref.shape[0])], axis=1)

  def start(copies):
    for cp in copies:
      cp.start()

  def wait(copies):
    for cp in copies:
      cp.wait()

  def rows_f32(ref, first):
    return ref[pl.ds(first, 16), :].astype(F32)

  unit_groups = lambda u: (2 * u, 2 * u + 1, 2 * u + 4, 2 * u + 5)
  cp_c = copy(c_hbm, c_v)
  cp_phi = copy(wphi_hbm, wphi_v)
  cp_wq, cp_wk = [[slab_copies(wqkv_hbm, wqkv_v.at[i], i * NJ, unit_groups(u))
                   for u in range(2)] for i in range(2)]
  cp_wv = [slab_copies(wqkv_hbm, wqkv_v.at[2], 2 * NJ, which)
           for which in (unit_groups(0), (2, 6), (3, 7))]
  cp_shift = slab_copies(wmod_hbm, wshift_v)
  cp_scale = [slab_copies(wmod_hbm, wscale_v, NJ, (j, j + 4)) for j in range(4)]
  cp_scale[3] = cp_wv[1] + cp_scale[3]
  cp_x = [copy(x_hbm.at[pl.ds(i * TM, TM)], x_v.at[pl.ds(i * TM, TM)]) for i in range(NT)]
  cp_late = ([cp_x[3]] + cp_wq[0] + cp_wq[1] + [copy(wr_hbm, wr_v)]
             + [copy(wmod_hbm.at[:, pl.ds(i * D, D)], wmod_v.at[i - 2]) for i in range(2, 6)]
             + [copy(wo_hbm, wo_v)])
  cp_wg = slab_copies(wg_hbm, wg_v)
  cp_wu = slab_copies(wu_hbm, wu_v)
  cp_wd = slab_copies(wd_hbm, wd_v)
  cp_out = [copy(out_v.at[pl.ds(n * TH, TH)], out_hbm.at[pl.ds(n * TH, TH)])
            for n in range(S // TH)]
  patch_sems = [next(sems), next(sems)]

  start([cp_c, cp_x[0]] + cp_wv[0] + sum(cp_scale, []) + cp_wv[2] + [cp_phi] + cp_wk[0]
        + cp_shift + [cp_x[1]] + cp_wk[1] + [cp_x[2]] + cp_late)

  stream = _Stream()
  mod = {}

  def block_diagonals():
    row = lax.broadcasted_iota(jnp.int32, (LANES, DH), 0)
    col = lax.broadcasted_iota(jnp.int32, (LANES, DH), 1)
    pick = jnp.where((row % PAIR) // 2 == col, 1.0, 0.0).astype(BF16)
    row = lax.broadcasted_iota(jnp.int32, (LANES, LANES), 0)
    col = lax.broadcasted_iota(jnp.int32, (LANES, LANES), 1)
    own_head = (row // PAIR) * 2 + row % 2 == col // DH
    return [jnp.where(own_head, _dot(pick, wphi_v[g * LANES:(g + 1) * LANES, :], TB),
                      0.0).astype(BF16) for g in range(NJ)]

  def fold_phi(which, u):
    def blocks(g, j):
      w = jnp.concatenate([wqkv_v[which, g, t * LANES:(t + 1) * LANES, :] for t in (j, j + 4)])
      return _lane_tiles(LOG2E * stream.product(bd[g], w, TB))
    return _assemble([[_left_operands(*blocks(g, j), *blocks(g + 4, j)) for j in range(4)]
                      for g in (2 * u, 2 * u + 1)])

  def value_weight(g, j):
    return wqkv_v[2, g, j * LANES:(j + 1) * LANES, :].astype(F32).T

  wo_parts = []

  def out_weight_piece(r, token):
    top, bot = _after(rows_f32(wo_v, r), token), rows_f32(wo_v, HALF + r)
    ops = _right_operands(top[:, :HALF], top[:, HALF:], bot[:, :HALF], bot[:, HALF:])
    wo_parts.append([ops])
    return _token(ops[0], ops[2], ops[5])

  def modulation_pieces(i):
    acc = []
    def piece(k, token):
      p = rows_f32(wmod_v.at[i - 2], k) * jnp.tile(_after(silu_col[k:k + 16], token), (1, NJ))
      p = p[0:8] + p[8:16]
      acc[:] = [acc[0] + p] if acc else [p]
      if k + 16 == D:
        mod[i] = jnp.sum(acc[0], axis=0, keepdims=True)
      return _token(acc[0]) if k % 64 == 48 else None
    return [(60, lambda t, k=k: piece(k, t)) for k in range(0, D, 16)]

  h_parts = [[] for _ in range(NT)]

  def modulate(i, top, bot):
    scale = 1.0 + mod[1]
    top = top * scale + mod[0]
    bot = bot * scale + mod[0]
    ops = _right_operands(top[:, :HALF], bot[:, :HALF], top[:, HALF:], bot[:, HALF:])
    h_parts[i].append([ops])
    return _token(ops[5], ops[6])

  def normalized_rows(first, token=None):
    return _normalize(_after(rows_f32(x_v, first), token))

  def prenorm_pieces(i):
    top = []
    def first(r, token):
      top.append(normalized_rows(i * TM + r, token))
    def second(r, token):
      return modulate(i, top.pop(), normalized_rows(i * TM + TH + r, token))
    return [(cost, lambda t, r=r, f=f: f(r, t))
            for r in range(0, TH, 16) for cost, f in ((120, first), (270, second))]

  def finish_prenorm(i, queue):
    while len(h_parts[i]) < TH // 16:
      queue.pop(0)[1](None)

  kv = [None] * NP
  z = [None] * NP
  keys, values = {}, {}

  def pairs_of(u, row):
    return [(8 * row + 4 * u + k, PAIR * k) for k in range(4)]

  def accumulate(acc, i, val):
    acc[i] = val if acc[i] is None else acc[i] + val

  def feature_pieces(u, row, block, cost, use):
    for pair, r in pairs_of(u, row):
      parts = []
      def piece(token, pair=pair, r=r, parts=parts):
        lo = len(parts) * LANES
        parts.append(_hedgehog(_after(block[r:r + PAIR, lo:lo + LANES], token)))
        use(pair, parts)
        return _token(parts[-1][7], parts[-1][15])
      stream.urgent += [(cost, piece)] * (TH // LANES)

  def joined(parts):
    return jnp.concatenate([jnp.concatenate(p, axis=0) for p in parts], axis=1)

  def combine(n, pair):
    if (n, pair) in keys and (n, pair) in values:
      def run():
        v = values[n, pair]
        if n < 2:
          v = v + jnp.tile(value_shift[pair * PAIR:(pair + 1) * PAIR], (1, TH // LANES))
        accumulate(kv, pair, _dot(v.astype(BF16), keys[n, pair], TB))
      stream.later(2, run)

  def keys_done(i, u, row, col, block):
    def use(pair, parts):
      if len(parts) == TH // LANES:
        phi = joined(parts)
        accumulate(z, pair, _tree(jnp.add, _lane_tiles(phi)))
        keys[2 * i + col, pair] = phi.astype(BF16)
        combine(2 * i + col, pair)
    feature_pieces(u, row, block, 125, use)

  def values_done(i, u, row, col, block):
    for pair, r in pairs_of(u, row):
      values[2 * i + col, pair] = block[r:r + PAIR]
      combine(2 * i + col, pair)

  def project(w, u, right, done, i):
    stream.block_product(w[u], right, TB, lambda *a: done(i, u, *a))

  cp_c.wait()
  c = jnp.broadcast_to(c_v[...].astype(F32), (16, D))
  silu_c = (c * jax.nn.sigmoid(c)).astype(BF16)
  silu_col = _columns(silu_c.astype(F32))

  cp_x[0].wait()
  for r in range(0, TM, 16):
    norm_v[pl.ds(r, 16), :] = normalized_rows(r)

  wait(cp_wv[0])
  first_wv = {(g, j): value_weight(g, j) for g in unit_groups(0) for j in range(NJ)}
  scales = [None] * NJ
  first_values = None
  for j in range(4):
    wait(cp_scale[j])
    both = _dot(silu_c, slabs(wscale_v, (j, j + 4)))
    scales[j], scales[j + 4] = _lane_tiles(both[0:1])
    lo, hi = [norm_v[:, t * LANES:(t + 1) * LANES] * (1.0 + scales[t]) for t in (j, j + 4)]
    for k, op in enumerate(_right_operands(lo[:TH], lo[TH:], hi[:TH], hi[TH:])):
      first_v[1, k, :, pl.ds(j * LANES, LANES)] = op.astype(BF16)
    w = jnp.concatenate([jnp.concatenate([first_wv[g, j], first_wv[g, j + 4]], axis=1)
                         for g in unit_groups(0)])
    term = _dot(w.astype(BF16), jnp.concatenate([lo, hi], axis=1).astype(BF16), TB)
    first_values = term if j == 0 else _after(first_values, both[0:8, 0:LANES]) + term
  mod[1] = jnp.concatenate(scales, axis=1)
  for row in range(2):
    for col in range(2):
      values_done(0, 0, row, col,
                  first_values[row * TH:(row + 1) * TH, col * TH:(col + 1) * TH])

  def store_value_weights(g):
    for j in range(4):
      ops = _left_operands(value_weight(g, j), value_weight(g, j + 4),
                           value_weight(g + 4, j), value_weight(g + 4, j + 4))
      for k, op in enumerate(ops):
        first_v[0, k, pl.ds(g % 2 * LANES, LANES), pl.ds(j * LANES, LANES)] = op.astype(BF16)

  store_value_weights(2)
  wait(cp_wv[2] + [cp_phi])
  store_value_weights(3)
  bd = block_diagonals()
  wv = [None, [first_v[0, k] for k in range(7)]]
  wv_parts = [[], []]

  def first_wv_piece(g, j, token):
    wv_parts[g].append(_left_operands(_after(first_wv[g, j], token), first_wv[g, j + 4],
                                      first_wv[g + 4, j], first_wv[g + 4, j + 4]))

  stream.relaxed += [(100, lambda t, g=g, j=j: first_wv_piece(g, j, t))
                     for g in range(2) for j in range(4)]
  project(wv, 1, [first_v[1, k] for k in range(7)], values_done, 0)
  stream.flush(stream.relaxed)

  wait(cp_wk[0])
  wk = [fold_phi(1, 0)]

  wait(cp_shift)
  shift = _dot(silu_c, slabs(wshift_v))
  mod[0] = shift[0:1]
  value_shift = _columns(_dot(shift.astype(BF16), slabs(wqkv_v.at[2])))
  for r in range(0, TH, 16):
    modulate(0, norm_v[pl.ds(r, 16), :], norm_v[pl.ds(TH + r, 16), :])
  h = [_assemble(h_parts[0])]
  project(wk, 0, h[0], keys_done, 0)

  wait(cp_x[1:3] + cp_wk[1])
  start(cp_wg)
  stream.urgent[:0] = prenorm_pieces(1)
  wk.append(fold_phi(1, 1))
  project(wk, 1, h[0], keys_done, 0)
  finish_prenorm(1, stream.urgent)
  wv[0] = _assemble(wv_parts)

  for i in range(1, NT):
    h.append(_assemble(h_parts[i]))
    if i > 1:
      for u in range(2):
        project(wk, u, h[i], keys_done, i)
    if i == 2:
      wait(cp_late)
      start(cp_wu + cp_wd)
      stream.relaxed += [p for k in range(2, 6) for p in modulation_pieces(k)]
      stream.relaxed += [(150, lambda t, r=r: out_weight_piece(r, t))
                         for r in range(0, HALF, 16)]
    if i + 1 < NT:
      stream.relaxed[:0] = prenorm_pieces(i + 1)
    for u in range(2):
      project(wv, u, h[i], values_done, i)
    if i == 1:
      for u in range(2):
        project(wk, u, h[i], keys_done, i)
    if i + 1 < NT:
      finish_prenorm(i + 1, stream.relaxed)

  wq = [fold_phi(0, u) for u in range(2)]
  stream.drain()
  row = lax.broadcasted_iota(jnp.int32, (PAIR, LANES), 0)
  col = lax.broadcasted_iota(jnp.int32, (PAIR, LANES), 1)
  own_head = row // DH == col % 2
  kv = [jnp.where(own_head, t, 0.0).astype(BF16) for t in kv]
  z = [jnp.broadcast_to(jnp.sum(t, axis=1, keepdims=True), (LANES, LANES)) for t in z]

  w_r = jnp.concatenate([wr_v[j:j + 1, :].astype(F32) for j in range(NJ)], axis=1)
  readout = {}
  o_parts = {}
  wo = []
  sublane = lax.broadcasted_iota(jnp.int32, (8, LANES), 0)
  best = [jnp.full((8, LANES), -jnp.inf, F32), jnp.full((8, LANES), S, jnp.int32)] * 2

  def readout_piece(n, g, token):
    lo, hi = [jnp.concatenate([t.T for t in _lane_tiles(_after(
        jnp.concatenate(readout[n, 2 * k] + readout[n, 2 * k + 1], axis=0), token))])
              for k in (g, g + 4)]
    o_parts[n, g] = _left_operands(lo[:LANES], hi[:LANES], lo[LANES:], hi[LANES:])

  def queries_done(i, u, row, col, block):
    n = 2 * i + col
    inv = {}
    def use(pair, parts):
      den = _per_head(jnp.add, [p * z[pair][8 * k:8 * k + 8] for k, p in enumerate(parts[-1])])
      inv.setdefault(pair, []).append(1.0 / (den + DEN_EPS))
      if len(parts) < TH // LANES:
        return
      phi = joined(parts).astype(BF16)
      def run():
        num = _dot(kv[pair], phi)
        scale = jnp.concatenate(inv[pair], axis=1)
        readout[n, pair] = [num[0:DH] * scale[0:1], num[DH:PAIR] * scale[1:2]]
        g = pair // 2 % 4
        if all((n, 2 * k + j) in readout for k in (g, g + 4) for j in range(2)):
          stream.urgent.append((150, lambda t: readout_piece(n, g, t)))
      stream.later(1, run)
    feature_pieces(u, row, block, 160, use)

  def finish_rows(first, attn, token):
    rows = pl.ds(first, 16)
    x1 = rows_f32(x_v, first) + mod[2] * _after(attn, token)
    h2 = _normalize(x1) * (1.0 + mod[4]) + mod[3]
    h2_v[rows, :] = h2.astype(BF16)
    out_v[rows, :] = (x1 + mod[5] * h2).astype(BF16)
    score = jnp.broadcast_to(jnp.sum(h2 * w_r, axis=1, keepdims=True), (16, LANES))
    for k in (0, 8):
      r, idx = score[k:k + 8], sublane + (first + k)
      m1, i1, m2, i2 = best
      over1, over2 = r > m1, r > m2
      best[:] = [jnp.where(over1, r, m1), jnp.where(over1, idx, i1),
                 jnp.where(over1, m1, jnp.where(over2, r, m2)),
                 jnp.where(over1, i1, jnp.where(over2, idx, i2))]
    if (first + 16) % TH == 0:
      cp_out[first // TH].start()
    return best[2]

  def output(n):
    if any((n, g) not in o_parts for g in range(4)):
      stream.drain()
    if not wo:
      stream.flush(stream.relaxed)
      wo.extend(_assemble(wo_parts))
    last = n == S // TH - 1
    blocks = {}
    def done(row, col, block):
      blocks[row, col] = block
      if (row, 1 - col) in blocks:
        for r in range(0, TH // 2, 16):
          attn = jnp.concatenate([blocks[row, 0][r:r + 16], blocks[row, 1][r:r + 16]], axis=1)
          first = n * TH + row * (TH // 2) + r
          stream.urgent.append((260, lambda t, s=first, a=attn: finish_rows(s, a, t)))
    if last:
      stream.rate = RATE * 5 // 4
    stream.block_product(_assemble([[o_parts[n, g] for g in range(4)]]), wo, NN, done, last)

  for i in range(NT + 1):
    if i < NT:
      for u in range(2):
        project(wq, u, h[i], queries_done, i)
    if i > 0:
      output(2 * i - 2)
      output(2 * i - 1)
  stream.drain()

  score = jnp.concatenate([best[0], best[2]], axis=0)
  idx = jnp.concatenate([best[1], best[3]], axis=0)
  m1 = jnp.max(score, axis=0, keepdims=True)
  i1 = jnp.min(jnp.where(score == m1, idx, S), axis=0, keepdims=True)
  score = jnp.where(idx == i1, -jnp.inf, score)
  m2 = jnp.max(score, axis=0, keepdims=True)
  i2 = jnp.min(jnp.where((score == m2) & (idx != i1), idx, S), axis=0, keepdims=True)
  tok1 = jnp.minimum(i1[0, 0], S - 1)
  tok2 = jnp.minimum(i2[0, 0], S - 1)
  sel = lax.broadcasted_iota(jnp.int32, (16, 1), 0)

  def group_of(tok):
    return pl.multiple_of((tok // 16) * 16, 16)

  def row_of(tok):
    rows = rows_f32(h2_v, group_of(tok))
    return jnp.sum(jnp.where(group_of(tok) + sel == tok, rows, 0.0), axis=0, keepdims=True)

  chosen = jnp.where(sel == 0, row_of(tok1), row_of(tok2)).astype(BF16)
  wait(cp_wg + cp_wu + cp_wd)

  down = [[None, None] for _ in range(NJ)]

  def down_piece(first, cols, token):
    hidden = [hidden_v[t, pl.ds(first, 16), :] for t in range(2)]
    hidden[0] = _after(hidden[0], token)
    for k in cols:
      w = rows_f32(wd_v.at[k], first)
      for t in range(2):
        part = w * hidden[t]
        accumulate(down[k], t, part[0:8] + part[8:16])

  stream.rate = RATE
  act = []
  for j in range(NF):
    gate, up = _lane_tiles(
        stream.product(chosen, jnp.concatenate([wg_v[j], wu_v[j]], axis=1), NN))
    act.append((gate * jax.nn.sigmoid(gate) * up).astype(BF16).astype(F32))
    if j < VECTOR_SLABS:
      for t in range(2):
        hidden_v[t, pl.ds(j * LANES, LANES), :] = _columns(act[j][t:t + 1])
      stream.urgent += [
          (44, lambda token, first=j * LANES + r, lo=lo:
           down_piece(first, range(lo, lo + 4), token))
          for lo in (0, 4) for r in range(0, LANES, 16)]
  y = None
  for j in range(VECTOR_SLABS, NF):
    part = stream.product(act[j].astype(BF16), slabs(wd_v, rows=pl.ds(j * LANES, LANES)), NN)
    y = part if y is None else y + part
  stream.drain()
  y += jnp.concatenate(
      [jnp.where(sel == 0, *[jnp.sum(t, axis=0, keepdims=True) for t in pair])
       for pair in down], axis=1)
  update = mod[5] * (y * jax.nn.sigmoid(jnp.where(sel == 0, m1[:, 0:1], m2[:, 0:1])))

  def patch(slot, tok):
    base = group_of(tok)
    rows = rows_f32(out_v, base)
    rows = jnp.where(base + sel == tok1, rows + update[0:1], rows)
    rows = jnp.where(base + sel == tok2, rows + update[1:2], rows)
    patch_v[slot] = rows.astype(BF16)
    return pltpu.make_async_copy(patch_v.at[slot], out_hbm.at[pl.ds(base, 16)],
                                 sem.at[patch_sems[slot]])

  cp1 = patch(0, tok1)
  cp2 = patch(1, tok2)
  wait(cp_out)
  cp1.start()

  @pl.when(tok1 // 16 != tok2 // 16)
  def _():
    cp2.start()
    cp2.wait()

  cp1.wait()


@jax.jit
def pallas_adaLN_cond__linear_kernel_hedgehog__moe_arch_mod__prompt_kernel(
    A_x: jax.Array,
    A_wqkv: jax.Array,
    A_w_phi: jax.Array,
    A_wo: jax.Array,
    B_x: jax.Array,
    B_w_r: jax.Array,
    B_w_gate: jax.Array,
    B_w_up: jax.Array,
    B_w_down: jax.Array,
    c: jax.Array,
    w_mod: jax.Array,
):
  del B_x
  scratch = [
      pltpu.VMEM((S, D), BF16),
      pltpu.VMEM((3, NJ, D, LANES), BF16),
      pltpu.VMEM((D, DH), BF16),
      pltpu.VMEM((D, D), BF16),
      pltpu.VMEM((NJ, LANES), BF16),
      pltpu.VMEM((NF, D, LANES), BF16),
      pltpu.VMEM((NF, D, LANES), BF16),
      pltpu.VMEM((NJ, F, LANES), BF16),
      pltpu.VMEM((1, D), BF16),
      pltpu.VMEM((4, D, D), BF16),
      pltpu.VMEM((NJ, D, LANES), BF16),
      pltpu.VMEM((NJ, D, LANES), BF16),
      pltpu.VMEM((TM, D), F32),
      pltpu.VMEM((2, 7, TH, HALF), BF16),
      pltpu.VMEM((S, D), BF16),
      pltpu.VMEM((S, D), BF16),
      pltpu.VMEM((2, VECTOR_SLABS * LANES, LANES), F32),
      pltpu.VMEM((2, 16, D), BF16),
      pltpu.SemaphoreType.DMA((40,)),
  ]
  out = pl.pallas_call(
      _kernel,
      out_shape=jax.ShapeDtypeStruct((S, D), BF16),
      in_specs=[pl.BlockSpec(memory_space=pl.ANY)] * 10,
      out_specs=pl.BlockSpec(memory_space=pl.ANY),
      scratch_shapes=scratch,
      compiler_params=pltpu.CompilerParams(vmem_limit_bytes=120 * 1024 * 1024),
  )(A_x.reshape(S, D), A_wqkv, A_w_phi.reshape(D, DH), A_wo, B_w_r.reshape(NJ, LANES),
    B_w_gate, B_w_up, B_w_down, c, w_mod)
  return out.reshape(1, S, D)
```
